```python
import os as _os
_os.environ.setdefault("JAX_PLATFORMS", "cpu")
import jax
import jax.numpy as jnp

def _softmax(x, axis=-1):
    return jax.nn.softmax(x, axis=axis)
def _gelu(x):
    return jax.nn.gelu(x, approximate=True)
def _silu(x):
    return jax.nn.silu(x)
def _sigmoid(x):
    return jax.nn.sigmoid(x)
def _layernorm(x, axis=-1, eps=1e-5):
    m = jnp.mean(x, axis=axis, keepdims=True)
    v = jnp.var(x, axis=axis, keepdims=True)
    return (x - m) / jnp.sqrt(v + eps)
def _scatter_add(tgt, idx, src, axis=0):
    return tgt.at[idx].add(src)
def _segment_sum(src, seg, n):
    return jax.ops.segment_sum(src, seg, n)
class _Rng:
    def __init__(self, key):
        self._k = key
    def _next(self):
        self._k, sub = jax.random.split(self._k)
        return sub
    def normal(self, shape):
        return jax.random.normal(self._next(), shape, dtype=jnp.bfloat16)
    def randint(self, lo, hi, shape):
        return jax.random.randint(self._next(), shape, lo, hi, dtype=jnp.int32)
    def uniform(self, shape, lo=0.0, hi=1.0):
        return jax.random.uniform(self._next(), shape, jnp.bfloat16, lo, hi)
    def permutation(self, n):
        return jax.random.permutation(self._next(), n)


kernel_name = 'standalone__linear_kernel_hedgehog__prompt'

def setup_inputs():
    _rng = _Rng(jax.random.key(int.from_bytes(__import__("os").urandom(4), "little")))
    _w = (lambda a: (lambda t: t.astype(jnp.bfloat16) if jnp.issubdtype(t.dtype, jnp.floating) else t)(jnp.asarray(a)))
    B, S, D, H = 1, 2048, 1024, 32
    Dh = D // H
    return {
        "x": _w((lambda *s: _rng.normal(s) * 0.4)(B, S, D)),
        "wqkv": _w((lambda *s: _rng.normal(s) * 0.4)(D, 3 * D)),
        "w_phi": _w((lambda *s: _rng.normal(s) * 0.4)(H, Dh, Dh) * (Dh ** -0.5)),
        "wo": _w((lambda *s: _rng.normal(s) * 0.05)(D, D)),
    }

def reference(x, wqkv, w_phi, wo):
    B, S, D = x.shape
    H = 32; Dh = D // H
    qkv = (lambda x, *d: x.transpose(*d))((x @ wqkv).reshape(B, S, 3, H, Dh), 2, 0, 3, 1, 4)
    q, k, v = qkv[0], qkv[1], qkv[2]
    pq = jnp.einsum("bhsd,hdf->bhsf", q, w_phi)
    pk = jnp.einsum("bhsd,hdf->bhsf", k, w_phi)
    phi_q = jnp.concatenate([_softmax(pq, axis=-1), _softmax(-pq, axis=-1)], axis=-1)
    phi_k = jnp.concatenate([_softmax(pk, axis=-1), _softmax(-pk, axis=-1)], axis=-1)
    kv = jnp.einsum("bhsf,bhsd->bhfd", phi_k, v)
    z  = jnp.einsum("bhsf->bhf", phi_k)
    num = jnp.einsum("bhqf,bhfd->bhqd", phi_q, kv)
    den = jnp.einsum("bhqf,bhf->bhq", phi_q, z)[..., None] + 1e-6
    o = num / den
    return (lambda x, *d: x.transpose(*d))(o, 0, 2, 1, 3).reshape(B, S, D) @ wo
```

```python
import functools
import contextlib
import jax
import jax.numpy as jnp
from jax import lax
import jax.experimental.pallas as pl
import jax.experimental.pallas.tpu as pltpu

S, D, H, DH = 2048, 1024, 32, 32
LOG2E = 1.4426950408889634
F32, BF16 = jnp.float32, jnp.bfloat16
NT = (((1,), (1,)), ((), ()))


def dot_nt(a, b):
    return lax.dot_general(a, b, NT, preferred_element_type=F32)


def dot_nn(a, b):
    return jnp.dot(a, b, preferred_element_type=F32)


def allred(x, op):
    y = op(op(x[0:8], x[8:16]), op(x[16:24], x[24:32]))
    for sh in (4, 2, 1):
        y = op(y, pltpu.roll(y, sh, 0))
    return y


def rep4(y):
    return jnp.concatenate([y] * 4, axis=0)


def make(TS=512, GK=2, GQ=256, OC=4, vz=True, prof=False, interpret=False, unroll1=False, unroll2=False):
    nT = S // TS
    ON = D // OC
    LR = 64 if vz else 80
    scope = jax.named_scope if prof else (lambda name: contextlib.nullcontext())

    def softpm(ph):
        mx = rep4(allred(ph, jnp.maximum))
        mn = rep4(allred(ph, jnp.minimum))
        ep = jnp.exp2(ph - mx)
        en = jnp.exp2(mn - ph)
        rp = 1.0 / allred(ep, jnp.add)
        rn = 1.0 / allred(en, jnp.add)
        return ep, en, rp, rn

    def kernel(x_hbm, w_hbm, wphi_hbm, wo_hbm, o_hbm,
               xs, wst, wphis, wos, wT, bds, acc, A, lhs, phi, oT, ost, zacc,
               sem_x, sem_w, sem_m, sem_o):
        def cp_w(c):
            return pltpu.make_async_copy(w_hbm.at[:, pl.ds(128 * c, 128)], wst.at[c], sem_w.at[c])

        def cp_x(t):
            s0 = pl.multiple_of(t * TS, TS)
            return pltpu.make_async_copy(x_hbm.at[pl.ds(s0, TS), :], xs.at[pl.ds(s0, TS), :], sem_x.at[t])

        def cp_o(t, c):
            s0 = pl.multiple_of(t * TS, TS)
            return pltpu.make_async_copy(ost.at[pl.ds(s0, TS), pl.ds(ON * c, ON)],
                                         o_hbm.at[pl.ds(s0, TS), pl.ds(ON * c, ON)], sem_o.at[t * OC + c])

        cp_phi0 = pltpu.make_async_copy(wphi_hbm.at[pl.ds(0, 8)], wphis.at[pl.ds(0, 8)], sem_m.at[0])
        cp_phi1 = pltpu.make_async_copy(wphi_hbm.at[pl.ds(8, 24)], wphis.at[pl.ds(8, 24)], sem_m.at[2])
        cp_wo = pltpu.make_async_copy(wo_hbm, wos, sem_m.at[1])

        def kr(g):
            return D + 256 * g

        def vr(g):
            return D + 256 * g + 128

        cp_phi0.start()
        cp_w(8).start()
        cp_x(0).start()
        cp_w(16).start()
        cp_w(9).start(priority=1)
        cp_w(17).start(priority=1)
        cp_phi1.start(priority=1)

        if not vz:
            for j in range(16):
                lhs[j, 64:80, :] = jnp.ones((16, TS), BF16)
        row = lax.broadcasted_iota(jnp.int32, (128, 128), 0)
        col = lax.broadcasted_iota(jnp.int32, (128, 128), 1)
        bdmask = (row // 32) == (col // 32)

        def make_bd(g):
            w4 = wphis[4 * g:4 * g + 4].astype(F32).reshape(128, 32)
            bd = jnp.where(bdmask, jnp.concatenate([w4] * 4, axis=1), 0.0)
            bds[g] = bd.T.astype(BF16)

        def fold(c, g, r0):
            wT[r0:r0 + 128, :] = (dot_nt(bds[g], wst[c]) * LOG2E).astype(BF16)

        def trans_v(g):
            wT[vr(g):vr(g) + 128, :] = wst[16 + g].T

        def feat_k(p, r0, first):
            for h in range(p.shape[0] // 32):
                ep, en, rp, rn = softpm(p[32 * h:32 * h + 32, :])
                for e, r, o in ((ep, rp, 0), (en, rn, 32)):
                    f = e * rep4(r)
                    a = r0 + 64 * h + o
                    phi[a:a + 32, :] = f.astype(BF16)
                    if vz:
                        zp = f[:, 0:128]
                        for l in range(1, TS // 128):
                            zp = zp + f[:, 128 * l:128 * l + 128]
                        zacc[a:a + 32, :] = zp if first else zacc[a:a + 32, :] + zp

        def feat_q(p, r0):
            for h in range(p.shape[0] // 32):
                ep, en, rp, rn = softpm(p[32 * h:32 * h + 32, :])
                a = r0 + 64 * h
                if vz:
                    zp = jnp.concatenate([zacc[a:a + 32, :]] * (TS // 128), axis=1)
                    zn = jnp.concatenate([zacc[a + 32:a + 64, :]] * (TS // 128), axis=1)
                    tp = ep * zp
                    tn = en * zn
                    tp = (tp[0:8] + tp[8:16]) + (tp[16:24] + tp[24:32])
                    tn = (tn[0:8] + tn[8:16]) + (tn[16:24] + tn[24:32])
                    den = tp * rp + tn * rn
                    for sh in (4, 2, 1):
                        den = den + pltpu.roll(den, sh, 0)
                    rd = 1.0 / (den + 1e-6)
                    rp = rp * rd
                    rn = rn * rd
                phi[a:a + 32, :] = (ep * rep4(rp)).astype(BF16)
                phi[a + 32:a + 64, :] = (en * rep4(rn)).astype(BF16)

        def store_v(v, g):
            v = v.astype(BF16)
            for jj in range(2):
                lhs[2 * g + jj, 0:64, :] = v[64 * jj:64 * jj + 64, :]

        with scope("tile0"):
            xt = lambda: xs[0:TS, :]
            cp_phi0.wait()
            make_bd(0)
            make_bd(1)
            cp_w(8).wait()
            fold(8, 0, kr(0))
            cp_x(0).wait()
            for g in (2, 3):
                cp_w(8 + g).start()
                cp_w(16 + g).start()
            p = dot_nt(wT[kr(0):kr(0) + 128, :], xt())
            cp_w(16).wait()
            trans_v(0)
            feat_k(p, 0, True)
            store_v(dot_nt(wT[vr(0):vr(0) + 128, :], xt()), 0)
            for g in range(1, 8):
                if g in (1, 2):
                    cp_w(8 + g).wait()
                    cp_w(16 + g).wait()
                elif g in (3, 5):
                    for gg in ((3, 4) if g == 3 else (5, 6, 7)):
                        cp_w(8 + gg).wait()
                        cp_w(16 + gg).wait()
                if g == 1:
                    cp_phi1.wait()
                    for gg in range(4, 8):
                        cp_w(8 + gg).start()
                        cp_w(16 + gg).start()
                if g == 2 and nT > 1:
                    cp_x(1).start()
                if g == 3:
                    for t in range(2, nT):
                        cp_x(t).start()
                if g == 5:
                    for gg in range(8):
                        cp_w(gg).start()
                    cp_wo.start()
                fold(8 + g, g, kr(g))
                trans_v(g)
                if g == 1:
                    for gg in range(2, 8):
                        make_bd(gg)
                if g >= 2:
                    store_v(dot_nt(wT[vr(g - 1):vr(g - 1) + 128, :], xt()), g - 1)
                    feat_k(p, 256 * (g - 1), True)
                p = dot_nt(wT[kr(g):kr(g) + 128, :], xt())
            store_v(dot_nt(wT[vr(7):vr(7) + 128, :], xt()), 7)
            feat_k(p, 256 * 7, True)
            for j in range(16):
                acc[j] = dot_nt(lhs[j], phi[128 * j:128 * j + 128, :])

        def ph1(t, _):
            s0 = pl.multiple_of(t * TS, TS)
            cp_x(t).wait()
            xt = xs[pl.ds(s0, TS), :]
            for g0 in range(0, 8, GK):
                pv = dot_nt(wT[kr(g0):kr(g0) + 256 * GK, :], xt)
                for g in range(g0, g0 + GK):
                    o = 256 * (g - g0)
                    feat_k(pv[o:o + 128], 256 * g, False)
                    store_v(pv[o + 128:o + 256], g)
            for j in range(16):
                acc[j] = acc[j] + dot_nt(lhs[j], phi[128 * j:128 * j + 128, :])
            return 0

        with scope("ph1"):
            if unroll1:
                for t in range(1, nT):
                    ph1(t, 0)
            else:
                lax.fori_loop(1, nT, ph1, 0)

        with scope("mid"):
            for g in range(8):
                cp_w(g).wait()
            if vz:
                ones = jnp.ones((128, 128), BF16)
                for j in range(16):
                    zacc[128 * j:128 * j + 128, :] = dot_nn(
                        zacc[128 * j:128 * j + 128, :].astype(BF16), ones)
            for g in range(8):
                fold(g, g, 128 * g)
            rr = lax.broadcasted_iota(jnp.int32, (LR, 128), 0)
            cc = lax.broadcasted_iota(jnp.int32, (LR, 128), 1)
            rh = rr // 32 if vz else jnp.where(rr < 64, rr // 32, (rr - 64) // 8)
            amask = rh == (cc // 64)
            for j in range(16):
                A[j] = jnp.where(amask, acc[j], 0.0).astype(BF16)
            cp_wo.wait()

        def ph2(t, _):
            s0 = pl.multiple_of(t * TS, TS)
            xt = xs[pl.ds(s0, TS), :]
            for g in range(D // GQ):
                p = dot_nt(wT[GQ * g:GQ * g + GQ, :], xt)
                feat_q(p, 2 * GQ * g)
            for j in range(16):
                nd = dot_nn(A[j], phi[128 * j:128 * j + 128, :])
                if vz:
                    oT[64 * j:64 * j + 64, :] = nd.astype(BF16)
                else:
                    for hh in range(2):
                        rden = 1.0 / (nd[64 + 8 * hh:72 + 8 * hh, :] + 1e-6)
                        rden = jnp.concatenate([rden] * 4, axis=0)
                        oT[64 * j + 32 * hh: 64 * j + 32 * hh + 32, :] = (
                            nd[32 * hh:32 * hh + 32, :] * rden).astype(BF16)
            o = oT[...].T
            for c in range(OC):
                ost[pl.ds(s0, TS), ON * c:ON * c + ON] = dot_nn(o, wos[:, ON * c:ON * c + ON]).astype(BF16)
                cp_o(t, c).start()
            return 0

        with scope("ph2"):
            if unroll2:
                for t in range(nT):
                    ph2(t, 0)
            else:
                lax.fori_loop(0, nT, ph2, 0)
        with scope("tail"):
            for t in range(nT):
                for c in range(OC):
                    cp_o(t, c).wait()

    @jax.jit
    def fn(x, wqkv, w_phi, wo):
        anyspec = pl.BlockSpec(memory_space=pl.ANY)
        out = pl.pallas_call(
            kernel,
            out_shape=jax.ShapeDtypeStruct((S, D), BF16),
            in_specs=[anyspec] * 4,
            out_specs=anyspec,
            scratch_shapes=[
                pltpu.VMEM((S, D), BF16), pltpu.VMEM((24, D, 128), BF16),
                pltpu.VMEM((H, DH, DH), BF16), pltpu.VMEM((D, D), BF16),
                pltpu.VMEM((3 * D, D), BF16), pltpu.VMEM((8, 128, 128), BF16),
                pltpu.VMEM((16, LR, 128), F32), pltpu.VMEM((16, LR, 128), BF16),
                pltpu.VMEM((16, LR, TS), BF16), pltpu.VMEM((2 * D, TS), BF16),
                pltpu.VMEM((D, TS), BF16), pltpu.VMEM((S, D), BF16),
                pltpu.VMEM((2 * D, 128), F32),
                pltpu.SemaphoreType.DMA((nT,)), pltpu.SemaphoreType.DMA((24,)),
                pltpu.SemaphoreType.DMA((3,)), pltpu.SemaphoreType.DMA((nT * OC,)),
            ],
            compiler_params=pltpu.CompilerParams(vmem_limit_bytes=100 * 1024 * 1024),
            interpret=interpret,
        )(x.reshape(S, D), wqkv, w_phi, wo)
        return out.reshape(1, S, D)

    return fn


_impl = make(vz=False, GK=1)


@jax.jit
def pallas_standalone__linear_kernel_hedgehog__prompt_kernel(x, wqkv, w_phi, wo):
    return _impl(x, wqkv, w_phi, wo)
```

```python
import functools
import contextlib
import jax
import jax.numpy as jnp
from jax import lax
import jax.experimental.pallas as pl
import jax.experimental.pallas.tpu as pltpu

S, D, H, DH = 2048, 1024, 32, 32
LOG2E = 1.4426950408889634
F32, BF16, U32 = jnp.float32, jnp.bfloat16, jnp.uint32
NT = (((1,), (1,)), ((), ()))


def dot_nt(a, b):
    return lax.dot_general(a, b, NT, preferred_element_type=F32)


def dot_nn(a, b):
    return jnp.dot(a, b, preferred_element_type=F32)


def vregs(x):
    return [x[8 * i:8 * i + 8] for i in range(x.shape[0] // 8)]


def tree(op, xs):
    while len(xs) > 1:
        xs = [op(xs[i], xs[i + 1]) for i in range(0, len(xs), 2)]
    return xs[0]


def allred(x, op):
    y = tree(op, vregs(x))
    for sh in (4, 2):
        y = op(y, pltpu.roll(y, sh, 0))
    return y


def rep(y, n):
    return jnp.concatenate([y] * n, axis=0)


def lcat(pieces):
    return pieces[0] if len(pieces) == 1 else jnp.concatenate(pieces, axis=1)


def upk(x):
    return pltpu.bitcast(x, BF16)


def pk(x):
    return pltpu.bitcast(x, U32)


def pack_rows(f):
    v = vregs(f)
    return jnp.concatenate(
        [pltpu.bitcast(pltpu.pack_elementwise([v[i], v[i + 1]], packed_dtype=BF16), U32)
         for i in range(0, len(v), 2)], axis=0)


def make(TS=512, GK=1, GQ=256, OC=4, vz=False, prof=False, interpret=False, ORD=0, frcp=True, uphi=True, uw=True, TS2=512, BD=1, TV=0, ST=0, NX0=1, nochk=False, nodma=False, ZT=0, flags=None, AN=0):
    nT = S // TS
    nL = TS // 128
    ON = D // OC
    LR = 64 if vz else 80
    scope = jax.named_scope if prof else (lambda name: contextlib.nullcontext())

    def rcp(x):
        if frcp:
            return pl.reciprocal(x, approx=False, full_range=False)
        return 1.0 / x

    def softpm(ph):
        mx = rep(allred(ph, jnp.maximum), 8)
        mn = rep(allred(ph, jnp.minimum), 8)
        ep = jnp.exp2(ph - mx)
        en = jnp.exp2(mn - ph)
        rp = rcp(allred(ep, jnp.add))
        rn = rcp(allred(en, jnp.add))
        return ep, en, rp, rn

    def kernel(x_hbm, w_hbm, wphi_hbm, wo_hbm, o_hbm,
               xs, wst, wphis, wos, wT, bds, acc, A, lhs, phi, oT, ost, zacc, anch,
               sem_x, sem_w, sem_o, sem_b):
        (S_A, S_X0, S_B1, S_B2, S_B3, S_B5, S_Q, S_K0, S_V0) = (0, 1, 1 + NX0, 2 + NX0, 3 + NX0, 4 + NX0, 5 + NX0, 6 + NX0, 7 + NX0)
        if ST == 0:
            slot = {8: S_K0, 16: S_B1, 9: S_B1, 17: S_B2, 10: S_B2, 18: S_B3, 11: S_B3, 19: S_B3, 12: S_B3}
        else:
            slot = {8: S_K0, 16: S_V0, 9: S_B1, 17: S_B2, 10: S_B2, 18: S_B3, 11: S_B3, 19: S_B3, 12: S_B3}
        for c in (20, 21, 22, 23, 13, 14, 15):
            slot[c] = S_B5
        for c in range(8):
            slot[c] = S_Q

        def cp_w(c):
            return pltpu.make_async_copy(w_hbm.at[:, pl.ds(128 * c, 128)], wst.at[c].bitcast(BF16), sem_w.at[slot[c]])

        def cp_x0(q):
            n = 8 // NX0
            return [pltpu.make_async_copy(x_hbm.at[pl.ds(0, TS), pl.ds(128 * j, 128)],
                                          xs.at[j, pl.ds(0, TS // 2), :].bitcast(BF16), sem_w.at[S_X0 + q])
                    for j in range(n * q, n * q + n)]

        def cp_x(t):
            s0 = pl.multiple_of(t * TS, TS)
            h0 = pl.multiple_of(t * (TS // 2), TS // 2)
            return [pltpu.make_async_copy(x_hbm.at[pl.ds(s0, TS), pl.ds(128 * j, 128)],
                                          xs.at[j, pl.ds(h0, TS // 2), :].bitcast(BF16), sem_x.at[t - 1]) for j in range(8)]

        def cp_o(t, c):
            s0 = pl.multiple_of(t * TS2, TS2)
            return pltpu.make_async_copy(ost.at[pl.ds(s0, TS2), pl.ds(ON * c, ON)],
                                         o_hbm.at[pl.ds(s0, TS2), pl.ds(ON * c, ON)], sem_o.at[0])

        cp_phi0 = pltpu.make_async_copy(wphi_hbm.at[pl.ds(0, 12)], wphis.at[pl.ds(0, 12)], sem_w.at[S_A])
        cp_phi1 = pltpu.make_async_copy(wphi_hbm.at[pl.ds(12, 20)], wphis.at[pl.ds(12, 20)], sem_w.at[S_B2])
        cp_wo = [pltpu.make_async_copy(wo_hbm.at[:, pl.ds(128 * j, 128)], wos.at[j].bitcast(BF16), sem_w.at[S_Q])
                 for j in range(8)]

        def fence():
            pl.semaphore_signal(sem_b, 1)
            pl.semaphore_wait(sem_b, 1)

        def start(cps):
            for c in cps:
                c.start()
            fence()

        wcount = [0]

        def wait(cps, name=None):
            wcount[0] += 1
            with scope(f"w{wcount[0]:02d}_{name}"):
                for c in cps:
                    c.wait()

        def kr(g):
            return D + 256 * g

        def vr(g):
            return D + 256 * g + 128

        def xtile(h0, ts=TS):
            return lcat([upk(xs[j, pl.ds(h0, ts // 2), :]) for j in range(8)])

        def wrows(r0, n):
            return upk(wT[r0 // 2:(r0 + n) // 2, :]) if uw else wT[r0:r0 + n, :]

        def put_wT(r0, val):
            if uw:
                wT[r0 // 2:r0 // 2 + 64, :] = pk(val)
            else:
                wT[r0:r0 + 128, :] = val

        def put_phi(a, f):
            n = f.shape[1]
            if uphi:
                phi[a // 2:a // 2 + 32, 0:n] = pack_rows(f)
            else:
                phi[a:a + 64, 0:n] = f.astype(BF16)

        def get_phi(j, n=TS):
            return upk(phi[64 * j:64 * j + 64, 0:n]) if uphi else phi[128 * j:128 * j + 128, 0:n]

        start([cp_phi0])
        start([cp_w(8)])
        if ST == 1:
            start([cp_w(16)])
        for q in range(NX0):
            start(cp_x0(q))
        if ST == 0:
            start([cp_w(16)])
        start([cp_w(9)])
        start([cp_w(17)])
        start([cp_phi1])
        for g in range(2, 8):
            start([cp_w(8 + g)])
            start([cp_w(16 + g)])
        for t in range(1, nT):
            start(cp_x(t))
        start([cp_w(g) for g in range(8)])
        start(cp_wo)

        if not vz:
            for j in range(16):
                lhs[j, 64:80, :] = jnp.ones((16, TS), BF16)
        row = lax.broadcasted_iota(jnp.int32, (128, 128), 0)
        col = lax.broadcasted_iota(jnp.int32, (128, 128), 1)
        bdmask = (row // 32) == (col // 32)
        src = (row // 64) * 64 + (row % 2) * 32 + ((row % 64) // 8) * 4 + (row % 8) // 2
        perm = jnp.where(src == col, 1.0, 0.0).astype(BF16)

        def make_bd(g):
            w4 = wphis[4 * g:4 * g + 4].astype(F32).reshape(128, 32)
            bd = jnp.where(bdmask, jnp.concatenate([w4] * 4, axis=1), 0.0).astype(BF16)
            bds[g] = dot_nt(perm, bd).astype(BF16)

        def fold(c, g, r0):
            put_wT(r0, (dot_nt(bds[g], upk(wst[c])) * LOG2E).astype(BF16))

        def trans_v(g):
            put_wT(vr(g), upk(wst[16 + g]).T)

        def feat_k(p, r0, first):
            for j in range(p.shape[0] // 64):
                ep, en, rp, rn = softpm(p[64 * j:64 * j + 64, :])
                for e, r, o in ((ep, rp, 0), (en, rn, 64)):
                    f = e * rep(r, 8)
                    a = r0 + 128 * j + o
                    put_phi(a, f)
                    if vz:
                        zp = f[:, 0:128]
                        for l in range(1, nL):
                            zp = zp + f[:, 128 * l:128 * l + 128]
                        zacc[a:a + 64, :] = zp if first else zacc[a:a + 64, :] + zp

        def feat_q(p, r0):
            for j in range(p.shape[0] // 64):
                ep, en, rp, rn = softpm(p[64 * j:64 * j + 64, :])
                a = r0 + 128 * j
                if vz:
                    tp = tree(jnp.add, vregs(ep * lcat([zacc[a:a + 64, :]] * (TS2 // 128))))
                    tn = tree(jnp.add, vregs(en * lcat([zacc[a + 64:a + 128, :]] * (TS2 // 128))))
                    den = tp * rp + tn * rn
                    for sh in (4, 2):
                        den = den + pltpu.roll(den, sh, 0)
                    rd = rcp(den + 1e-6)
                    rp = rp * rd
                    rn = rn * rd
                put_phi(a, ep * rep(rp, 8))
                put_phi(a + 64, en * rep(rn, 8))

        def store_v(v, g):
            v = v.astype(BF16)
            for jj in range(2):
                lhs[2 * g + jj, 0:64, :] = v[64 * jj:64 * jj + 64, :]

        def kv_dot(j):
            return dot_nt(lhs[j], get_phi(j))

        with scope("tile0"):
            xt = lambda: xtile(0)
            projk = lambda g: dot_nt(wrows(kr(g), 128), xt())
            projv = lambda g: store_v(dot_nt(wrows(vr(g), 128), xt()), g)
            wait([cp_phi0], 'a')
            make_bd(0)
            make_bd(1)
            make_bd(2)
            wait([cp_w(8)], 'k0')
            fold(8, 0, kr(0))
            if ST == 1:
                wait([cp_w(16)], 'v0')
                trans_v(0)
            kq = D // NX0
            p = None
            for q in range(NX0):
                wait(cp_x0(q), 'x0')
                n = 8 // NX0
                xq = lcat([upk(xs[j, 0:TS // 2, :]) for j in range(n * q, n * q + n)])
                wq_ = wrows(kr(0), 256 if ST == 1 else 128)[:, kq * q:kq * q + kq]
                pq_ = dot_nt(wq_, xq)
                p = pq_ if p is None else p + pq_
            if ST == 1:
                store_v(p[128:256], 0)
                p = p[0:128]
            for g in range(1, 8):
                if AN and g in (1, 2, 3, 5):
                    anch[...] = p[120:128, TS - 128:TS] if AN == 1 else p[0:8, 0:128]
                if g == 1:
                    wait(([cp_w(16)] if ST == 0 else []) + [cp_w(9)], 'b1')
                elif g == 2:
                    wait([cp_w(17), cp_phi1, cp_w(10)], 'b2')
                elif g == 3:
                    wait([cp_w(18), cp_w(11), cp_w(19), cp_w(12)], 'b3')
                elif g == 5:
                    wait([cp_w(16 + gg) for gg in (4, 5, 6, 7)] + [cp_w(8 + gg) for gg in (5, 6, 7)], 'b5')
                if ORD == 0:
                    fold(8 + g, g, kr(g))
                    skipv = (ST == 1 and g == 1)
                    if not TV:
                        if not skipv:
                            trans_v(g - 1)
                    else:
                        for gg in {1: (0,), 2: (1,), 3: (2, 3), 5: (4, 5, 6, 7)}.get(g, ()):
                            if not skipv:
                                trans_v(gg)
                    if g == 2 and BD == 0:
                        for gg in range(3, 8):
                            make_bd(gg)
                    if not skipv:
                        projv(g - 1)
                    feat_k(p, 256 * (g - 1), True)
                    if g == 2 and BD == 1:
                        for gg in range(3, 8):
                            make_bd(gg)
                    p = projk(g)
                    if g == 2 and BD == 2:
                        for gg in range(3, 8):
                            make_bd(gg)
                elif ORD == 1:
                    trans_v(g - 1)
                    fold(8 + g, g, kr(g))
                    feat_k(p, 256 * (g - 1), True)
                    if g == 2:
                        for gg in range(3, 8):
                            make_bd(gg)
                    projv(g - 1)
                    p = projk(g)
            if not TV:
                trans_v(7)
            projv(7)
            feat_k(p, 256 * 7, True)
            for j in range(16):
                acc[j] = kv_dot(j)

        def ph1(t, _):
            h0 = pl.multiple_of(t * (TS // 2), TS // 2)
            wait(cp_x(t), 'xt')
            xt = xtile(h0)
            for g0 in range(0, 8, GK):
                pv = dot_nt(wrows(kr(g0), 256 * GK), xt)
                for g in range(g0, g0 + GK):
                    o = 256 * (g - g0)
                    feat_k(pv[o:o + 128], 256 * g, False)
                    store_v(pv[o + 128:o + 256], g)
            for j in range(16):
                acc[j] = acc[j] + kv_dot(j)
            return 0

        with scope("ph1"):
            lax.fori_loop(1, nT, ph1, 0)

        with scope("mid"):
            wait([pltpu.make_async_copy(w_hbm.at[:, pl.ds(0, 2 * D)], w_hbm.at[:, pl.ds(0, 2 * D)], sem_w.at[S_Q])], 'q')
            if vz:
                ones = jnp.ones((128, 128), BF16)
                for j in range(16):
                    if ZT == 0:
                        zacc[128 * j:128 * j + 128, :] = dot_nn(
                            zacc[128 * j:128 * j + 128, :].astype(BF16), ones)
                    else:
                        zr = dot_nt(ones[0:16], zacc[128 * j:128 * j + 128, :].astype(BF16))
                        zacc[128 * j:128 * j + 128, :] = rep(zr, 8).T
            for g in range(8):
                fold(g, g, 128 * g)
            rr = lax.broadcasted_iota(jnp.int32, (LR, 128), 0)
            cc = lax.broadcasted_iota(jnp.int32, (LR, 128), 1)
            rh = rr // 32 if vz else jnp.where(rr < 64, rr // 32, (rr - 64) // 8)
            ch = (cc // 2) % 2 if uphi else cc % 2
            amask = rh == ch
            for j in range(16):
                A[j] = jnp.where(amask, acc[j], 0.0).astype(BF16)

        def ph2(t, _):
            s0 = pl.multiple_of(t * TS2, TS2)
            h0 = pl.multiple_of(t * (TS2 // 2), TS2 // 2)
            xt = xtile(h0, TS2)
            for g in range(D // GQ):
                p = dot_nt(wrows(GQ * g, GQ), xt)
                feat_q(p, 2 * GQ * g)
            for j in range(16):
                nd = dot_nn(A[j], get_phi(j, TS2))
                if vz:
                    oT[64 * j:64 * j + 64, :] = nd.astype(BF16)
                else:
                    for hh in range(2):
                        rden = rcp(nd[64 + 8 * hh:72 + 8 * hh, :] + 1e-6)
                        oT[64 * j + 32 * hh: 64 * j + 32 * hh + 32, :] = (
                            nd[32 * hh:32 * hh + 32, :] * rep(rden, 4)).astype(BF16)
            o = oT[...].T
            for c in range(OC):
                js = range(c * ON // 128, (c + 1) * ON // 128)
                ost[pl.ds(s0, TS2), ON * c:ON * c + ON] = dot_nn(o, lcat([upk(wos[j]) for j in js])).astype(BF16)
                if not nodma:
                    cp_o(t, c).start()
            return 0

        with scope("ph2"):
            lax.fori_loop(0, S // TS2, ph2, 0)
        with scope("tail"):
            if not nodma:
                pltpu.make_async_copy(ost, ost, sem_o.at[0]).wait()

    @jax.jit
    def fn(x, wqkv, w_phi, wo):
        anyspec = pl.BlockSpec(memory_space=pl.ANY)
        out = pl.pallas_call(
            kernel,
            out_shape=jax.ShapeDtypeStruct((S, D), BF16),
            in_specs=[anyspec] * 4,
            out_specs=anyspec,
            scratch_shapes=[
                pltpu.VMEM((8, S // 2, 128), U32), pltpu.VMEM((24, D // 2, 128), U32),
                pltpu.VMEM((H, DH, DH), BF16), pltpu.VMEM((8, D // 2, 128), U32),
                pltpu.VMEM((3 * D // 2, D), U32) if uw else pltpu.VMEM((3 * D, D), BF16),
                pltpu.VMEM((8, 128, 128), BF16),
                pltpu.VMEM((16, LR, 128), F32), pltpu.VMEM((16, LR, 128), BF16),
                pltpu.VMEM((16, LR, TS), BF16),
                pltpu.VMEM((D, max(TS, TS2)), U32) if uphi else pltpu.VMEM((2 * D, max(TS, TS2)), BF16),
                pltpu.VMEM((D, TS2), BF16), pltpu.VMEM((S, D), BF16),
                pltpu.VMEM((2 * D, 128), F32), pltpu.VMEM((8, 128), F32),
                pltpu.SemaphoreType.DMA((nT - 1,)), pltpu.SemaphoreType.DMA((8 + NX0,)),
                pltpu.SemaphoreType.DMA((1,)),
                pltpu.SemaphoreType.REGULAR,
            ],
            compiler_params=pltpu.CompilerParams(vmem_limit_bytes=100 * 1024 * 1024, disable_semaphore_checks=nochk, disable_bounds_checks=nochk, flags=flags),
            interpret=interpret,
        )(x.reshape(S, D), wqkv, w_phi, wo)
        return out.reshape(1, S, D)

    return fn


_impl = make(vz=True, ZT=1, GQ=128, ST=1, NX0=4, nochk=True, OC=8)


@jax.jit
def pallas_standalone__linear_kernel_hedgehog__prompt_kernel(x, wqkv, w_phi, wo):
    return _impl(x, wqkv, w_phi, wo)
```

```python
import jax
import jax.numpy as jnp
from jax import lax
import jax.experimental.pallas as pl
import jax.experimental.pallas.tpu as pltpu

S, D, H, DH = 2048, 1024, 32, 32
TS = 512
NT_ = S // TS
NL = TS // 128
LOG2E = 1.4426950408889634
F32, BF16, U32 = jnp.float32, jnp.bfloat16, jnp.uint32
_NT = (((1,), (1,)), ((), ()))
XS = ((0, 1), (2, 3), (4, 5, 6, 7))


def _dot_nt(a, b):
    return lax.dot_general(a, b, _NT, preferred_element_type=F32)


def _dot_nn(a, b):
    return jnp.dot(a, b, preferred_element_type=F32)


def _vregs(x):
    return [x[8 * i:8 * i + 8] for i in range(x.shape[0] // 8)]


def _tree(op, xs):
    while len(xs) > 1:
        xs = [op(xs[i], xs[i + 1]) for i in range(0, len(xs), 2)]
    return xs[0]


def _allred(x, op):
    y = _tree(op, _vregs(x))
    for sh in (4, 2):
        y = op(y, pltpu.roll(y, sh, 0))
    return y


def _rep(y, n):
    return jnp.concatenate([y] * n, axis=0)


def _lcat(pieces):
    return pieces[0] if len(pieces) == 1 else jnp.concatenate(pieces, axis=1)


def _upk(x):
    return pltpu.bitcast(x, BF16)


def _pack_rows(f):
    v = _vregs(f)
    return jnp.concatenate(
        [pltpu.bitcast(pltpu.pack_elementwise([v[i], v[i + 1]], packed_dtype=BF16), U32)
         for i in range(0, len(v), 2)], axis=0)


def _rcp(x):
    return pl.reciprocal(x, approx=False, full_range=False)


def _softpm(ph):
    mx = _rep(_allred(ph, jnp.maximum), 8)
    mn = _rep(_allred(ph, jnp.minimum), 8)
    ep = jnp.exp2(ph - mx)
    en = jnp.exp2(mn - ph)
    return ep, en, _rcp(_allred(ep, jnp.add)), _rcp(_allred(en, jnp.add))


S_PHI0, S_K0, S_V0, S_X0, S_B1, S_B2, S_B3, S_B5, S_Q, S_WO, S_OUT, S_X = 0, 1, 2, 3, 6, 7, 8, 9, 10, 11, 12, 13
N_SEM = S_X + NT_ - 1
_W_SLOT = {8: S_K0, 16: S_V0, 9: S_B1, 17: S_B2, 10: S_B2, 18: S_B3, 11: S_B3, 19: S_B3, 12: S_B3}
_W_SLOT.update({c: S_B5 for c in (20, 21, 22, 23, 13, 14, 15)})
_W_SLOT.update({c: S_Q for c in range(8)})


def _kernel(x_hbm, w_hbm, wphi_hbm, wo_hbm, o_hbm,
            xs, wst, wphis, wos, wT, bds, bscr, acc, amat, lhs, phi, oT, ost, zacc, sems, sem_b):
    def cp_w(c):
        return pltpu.make_async_copy(w_hbm.at[:, pl.ds(128 * c, 128)], wst.at[c].bitcast(BF16), sems.at[_W_SLOT[c]])

    def cp_x0(q):
        return [pltpu.make_async_copy(x_hbm.at[pl.ds(0, TS), pl.ds(128 * j, 128)],
                                      xs.at[j, pl.ds(0, TS // 2), :].bitcast(BF16), sems.at[S_X0 + q])
                for j in XS[q]]

    def cp_x(t):
        s0 = pl.multiple_of(t * TS, TS)
        h0 = pl.multiple_of(t * (TS // 2), TS // 2)
        return [pltpu.make_async_copy(x_hbm.at[pl.ds(s0, TS), pl.ds(128 * j, 128)],
                                      xs.at[j, pl.ds(h0, TS // 2), :].bitcast(BF16), sems.at[S_X + t - 1])
                for j in range(8)]

    def cp_o(t, c):
        s0 = pl.multiple_of(t * TS, TS)
        return pltpu.make_async_copy(ost.at[pl.ds(s0, TS), pl.ds(128 * c, 128)],
                                     o_hbm.at[pl.ds(s0, TS), pl.ds(128 * c, 128)], sems.at[S_OUT])

    cp_phi0 = pltpu.make_async_copy(wphi_hbm.at[pl.ds(0, 12)], wphis.at[pl.ds(0, 12)], sems.at[S_PHI0])
    cp_phi1 = pltpu.make_async_copy(wphi_hbm.at[pl.ds(12, 20)], wphis.at[pl.ds(12, 20)], sems.at[S_B2])
    cp_wo = [pltpu.make_async_copy(wo_hbm.at[:, pl.ds(128 * j, 128)], wos.at[j].bitcast(BF16), sems.at[S_WO])
             for j in range(8)]

    def start(cps):
        for c in cps:
            c.start()
        pl.semaphore_signal(sem_b, 1)
        pl.semaphore_wait(sem_b, 1)

    def wait(cps):
        for c in cps:
            c.wait()

    def kr(g):
        return D + 256 * g

    def vr(g):
        return D + 256 * g + 128

    def xtile(h0):
        return _lcat([_upk(xs[j, pl.ds(h0, TS // 2), :]) for j in range(8)])

    def wrows(r0, n):
        return _upk(wT[r0 // 2:(r0 + n) // 2, :])

    def put_wT(r0, val):
        wT[r0 // 2:r0 // 2 + 64, :] = pltpu.bitcast(val, U32)

    def put_phi(a, f):
        phi[a // 2:a // 2 + 32, :] = _pack_rows(f)

    def get_phi(j):
        return _upk(phi[64 * j:64 * j + 64, :])

    start([cp_phi0])
    start([cp_w(8)])
    start([cp_w(16)])
    for q in range(len(XS)):
        start(cp_x0(q))
    start([cp_w(9)])
    start([cp_w(17)])
    start([cp_phi1])
    for g in range(2, 8):
        start([cp_w(8 + g)])
        start([cp_w(16 + g)])
    for t in range(1, NT_):
        start(cp_x(t))
    start([cp_w(g) for g in range(8)])
    start(cp_wo)

    row = lax.broadcasted_iota(jnp.int32, (128, 128), 0)
    col = lax.broadcasted_iota(jnp.int32, (128, 128), 1)
    bdmask = (row // 32) == (col // 32)

    def make_bd(g):
        w4 = wphis[4 * g:4 * g + 4].astype(F32).reshape(128, 32)
        bdT = jnp.where(bdmask, jnp.concatenate([w4] * 4, axis=1), 0.0).T
        for pj in range(2):
            for hh in range(2):
                r = 64 * pj + 32 * hh
                bscr[g % 2, pl.ds(64 * pj + hh, 32, stride=2), :] = bdT[r:r + 32, :]
        bds[g] = bscr[g % 2].astype(BF16)

    def fold(c, g, r0):
        put_wT(r0, (_dot_nt(bds[g], _upk(wst[c])) * LOG2E).astype(BF16))

    def trans_v(g):
        put_wT(vr(g), _upk(wst[16 + g]).T)

    def feat_k(p, r0, first):
        for j in range(p.shape[0] // 64):
            ep, en, rp, rn = _softpm(p[64 * j:64 * j + 64, :])
            for e, r, o in ((ep, rp, 0), (en, rn, 64)):
                f = e * _rep(r, 8)
                a = r0 + 128 * j + o
                put_phi(a, f)
                zp = f[:, 0:128]
                for l in range(1, NL):
                    zp = zp + f[:, 128 * l:128 * l + 128]
                zacc[a:a + 64, :] = zp if first else zacc[a:a + 64, :] + zp

    def feat_q(p, r0):
        for j in range(p.shape[0] // 64):
            ep, en, rp, rn = _softpm(p[64 * j:64 * j + 64, :])
            a = r0 + 128 * j
            tp = _tree(jnp.add, _vregs(ep * _lcat([zacc[a:a + 64, :]] * NL)))
            tn = _tree(jnp.add, _vregs(en * _lcat([zacc[a + 64:a + 128, :]] * NL)))
            den = tp * rp + tn * rn
            for sh in (4, 2):
                den = den + pltpu.roll(den, sh, 0)
            rd = _rcp(den + 1e-6)
            put_phi(a, ep * _rep(rp * rd, 8))
            put_phi(a + 64, en * _rep(rn * rd, 8))

    def store_v(v, g):
        v = v.astype(BF16)
        for jj in range(2):
            lhs[2 * g + jj] = v[64 * jj:64 * jj + 64, :]

    def kv_dot(j):
        return _dot_nt(lhs[j], get_phi(j))

    wait([cp_phi0])
    for g in range(3):
        make_bd(g)
    wait([cp_w(8)])
    fold(8, 0, kr(0))
    wait([cp_w(16)])
    trans_v(0)
    p = None
    for q in range(len(XS)):
        wait(cp_x0(q))
        xq = _lcat([_upk(xs[j, 0:TS // 2, :]) for j in XS[q]])
        pq = _dot_nt(wrows(kr(0), 256)[:, 128 * XS[q][0]:128 * XS[q][-1] + 128], xq)
        p = pq if p is None else p + pq
    store_v(p[128:256], 0)
    p = p[0:128]
    for g in range(1, 8):
        if g == 1:
            wait([cp_w(9)])
        elif g == 2:
            wait([cp_w(17), cp_phi1, cp_w(10)])
        elif g == 3:
            wait([cp_w(18), cp_w(11), cp_w(19), cp_w(12)])
        elif g == 5:
            wait([cp_w(c) for c in (20, 21, 22, 23, 13, 14, 15)])
        fold(8 + g, g, kr(g))
        if g > 1:
            trans_v(g - 1)
            store_v(_dot_nt(wrows(vr(g - 1), 128), xtile(0)), g - 1)
        feat_k(p, 256 * (g - 1), True)
        if g == 2:
            for gg in range(3, 8):
                make_bd(gg)
        p = _dot_nt(wrows(kr(g), 128), xtile(0))
    trans_v(7)
    store_v(_dot_nt(wrows(vr(7), 128), xtile(0)), 7)
    feat_k(p, 256 * 7, True)
    for j in range(16):
        acc[j] = kv_dot(j)

    def ph1(t, _):
        h0 = pl.multiple_of(t * (TS // 2), TS // 2)
        wait(cp_x(t))
        xt = xtile(h0)
        for g in range(8):
            pv = _dot_nt(wrows(kr(g), 256), xt)
            feat_k(pv[0:128], 256 * g, False)
            store_v(pv[128:256], g)
        for j in range(16):
            acc[j] = acc[j] + kv_dot(j)
        return 0

    lax.fori_loop(1, NT_, ph1, 0)

    wait([cp_w(g) for g in range(8)])
    wait(cp_wo)
    ones = jnp.ones((16, 128), BF16)
    for j in range(16):
        zr = _dot_nt(ones, zacc[128 * j:128 * j + 128, :].astype(BF16))
        zacc[128 * j:128 * j + 128, :] = _rep(zr, 8).T
    for g in range(8):
        fold(g, g, 128 * g)
    rr = lax.broadcasted_iota(jnp.int32, (64, 128), 0)
    cc = lax.broadcasted_iota(jnp.int32, (64, 128), 1)
    amask = (rr // 32) == ((cc // 2) % 2)
    for j in range(16):
        amat[j] = jnp.where(amask, acc[j], 0.0).astype(BF16)

    def ph2(t, _):
        s0 = pl.multiple_of(t * TS, TS)
        h0 = pl.multiple_of(t * (TS // 2), TS // 2)
        xt = xtile(h0)
        for g in range(8):
            feat_q(_dot_nt(wrows(128 * g, 128), xt), 256 * g)
        for j in range(16):
            oT[64 * j:64 * j + 64, :] = _dot_nn(amat[j], get_phi(j)).astype(BF16)
        o = oT[...].T
        for c in range(8):
            ost[pl.ds(s0, TS), 128 * c:128 * c + 128] = _dot_nn(o, _upk(wos[c])).astype(BF16)
            cp_o(t, c).start()
        return 0

    lax.fori_loop(0, NT_, ph2, 0)
    pltpu.make_async_copy(ost, ost, sems.at[S_OUT]).wait()


@jax.jit
def pallas_standalone__linear_kernel_hedgehog__prompt_kernel(x, wqkv, w_phi, wo):
    anyspec = pl.BlockSpec(memory_space=pl.ANY)
    out = pl.pallas_call(
        _kernel,
        out_shape=jax.ShapeDtypeStruct((S, D), BF16),
        in_specs=[anyspec] * 4,
        out_specs=anyspec,
        scratch_shapes=[
            pltpu.VMEM((8, S // 2, 128), U32),
            pltpu.VMEM((24, D // 2, 128), U32),
            pltpu.VMEM((H, DH, DH), BF16),
            pltpu.VMEM((8, D // 2, 128), U32),
            pltpu.VMEM((3 * D // 2, D), U32),
            pltpu.VMEM((8, 128, 128), BF16),
            pltpu.VMEM((2, 128, 128), F32),
            pltpu.VMEM((16, 64, 128), F32),
            pltpu.VMEM((16, 64, 128), BF16),
            pltpu.VMEM((16, 64, TS), BF16),
            pltpu.VMEM((D, TS), U32),
            pltpu.VMEM((D, TS), BF16),
            pltpu.VMEM((S, D), BF16),
            pltpu.VMEM((2 * D, 128), F32),
            pltpu.SemaphoreType.DMA((N_SEM,)),
            pltpu.SemaphoreType.REGULAR,
        ],
        compiler_params=pltpu.CompilerParams(vmem_limit_bytes=100 * 1024 * 1024, disable_semaphore_checks=True),
    )(x.reshape(S, D), wqkv, w_phi, wo)
    return out.reshape(1, S, D)
```

```python
import jax
import jax.numpy as jnp
from jax import lax
import jax.experimental.pallas as pl
import jax.experimental.pallas.tpu as pltpu

S, D, H, DH = 2048, 1024, 32, 32
TS = 512
NT_ = S // TS
NL = TS // 128
LOG2E = 1.4426950408889634
F32, BF16, U32 = jnp.float32, jnp.bfloat16, jnp.uint32
_NT = (((1,), (1,)), ((), ()))
XS = ((0, 1), (2, 3), (4, 5, 6, 7))


def _dot_nt(a, b):
    return lax.dot_general(a, b, _NT, preferred_element_type=F32)


def _dot_nn(a, b):
    return jnp.dot(a, b, preferred_element_type=F32)


def _vregs(x):
    return [x[8 * i:8 * i + 8] for i in range(x.shape[0] // 8)]


def _tree(op, xs):
    while len(xs) > 1:
        xs = [op(xs[i], xs[i + 1]) for i in range(0, len(xs), 2)]
    return xs[0]


def _allred(x, op):
    y = _tree(op, _vregs(x))
    for sh in (4, 2):
        y = op(y, pltpu.roll(y, sh, 0))
    return y


def _rep(y, n):
    return jnp.concatenate([y] * n, axis=0)


def _lcat(pieces):
    return pieces[0] if len(pieces) == 1 else jnp.concatenate(pieces, axis=1)


def _upk(x):
    return pltpu.bitcast(x, BF16)


def _pk(x):
    return pltpu.bitcast(x, U32)


def _rcp(x):
    return pl.reciprocal(x, approx=False, full_range=False)


def _softpm(ph):
    mx = _rep(_allred(ph, jnp.maximum), 8)
    mn = _rep(_allred(ph, jnp.minimum), 8)
    ep = jnp.exp2(ph - mx)
    en = jnp.exp2(mn - ph)
    return ep, en, _rcp(_allred(ep, jnp.add)), _rcp(_allred(en, jnp.add))


S_PHI0, S_K0, S_V0, S_X0, S_B1, S_B2, S_B3, S_B5, S_Q, S_WO, S_OUT, S_X = 0, 1, 2, 3, 6, 7, 8, 9, 10, 11, 12, 13
N_SEM = S_X + NT_ - 1
_W_SLOT = {8: S_K0, 16: S_V0, 9: S_B1, 17: S_B2, 10: S_B2, 18: S_B3, 11: S_B3, 19: S_B3, 12: S_B3}
_W_SLOT.update({c: S_B5 for c in (20, 21, 22, 23, 13, 14, 15)})
_W_SLOT.update({c: S_Q for c in range(8)})


def _kernel(x_hbm, w_hbm, wphi_hbm, wo_hbm, o_hbm,
            xs, wst, wphis, wos, wT, bds, bscr, acc, amat, lhs, phi, oT, ost, zacc, xu, sems, sem_b):
    def cp_w(c):
        return pltpu.make_async_copy(w_hbm.at[:, pl.ds(128 * c, 128)], wst.at[c], sems.at[_W_SLOT[c]])

    def cp_x0(q):
        return [pltpu.make_async_copy(x_hbm.at[pl.ds(0, TS), pl.ds(128 * j, 128)],
                                      xs.at[j, pl.ds(0, TS), :], sems.at[S_X0 + q])
                for j in XS[q]]

    def cp_x(t):
        s0 = pl.multiple_of(t * TS, TS)
        return [pltpu.make_async_copy(x_hbm.at[pl.ds(s0, TS), pl.ds(128 * j, 128)],
                                      xs.at[j, pl.ds(s0, TS), :], sems.at[S_X + t - 1])
                for j in range(8)]

    def cp_o(t, c):
        s0 = pl.multiple_of(t * TS, TS)
        return pltpu.make_async_copy(ost.at[pl.ds(s0, TS), pl.ds(128 * c, 128)],
                                     o_hbm.at[pl.ds(s0, TS), pl.ds(128 * c, 128)], sems.at[S_OUT])

    cp_phi0 = pltpu.make_async_copy(wphi_hbm.at[pl.ds(0, 12)], wphis.at[pl.ds(0, 12)], sems.at[S_PHI0])
    cp_phi1 = pltpu.make_async_copy(wphi_hbm.at[pl.ds(12, 20)], wphis.at[pl.ds(12, 20)], sems.at[S_B2])
    cp_wo = [pltpu.make_async_copy(wo_hbm.at[:, pl.ds(128 * j, 128)], wos.at[j], sems.at[S_WO])
             for j in range(8)]

    def start(cps):
        for c in cps:
            c.start()
        pl.semaphore_signal(sem_b, 1)
        pl.semaphore_wait(sem_b, 1)

    def wait(cps):
        for c in cps:
            c.wait()

    def kr(g):
        return D + 256 * g

    def vr(g):
        return D + 256 * g + 128

    def xtile(s0):
        return _lcat([xs[j, pl.ds(s0, TS), :] for j in range(8)])

    def wrows(r0, n):
        return _upk(wT[r0 // 2:(r0 + n) // 2, :])

    def put_wT(r0, val):
        wT[r0 // 2:r0 // 2 + 64, :] = _pk(val)

    def put_phi(a, f):
        phi[a // 2:a // 2 + 32, :] = _pk(f.astype(BF16))

    def get_phi(j):
        return _upk(phi[64 * j:64 * j + 64, :])

    start([cp_phi0])
    start([cp_w(8)])
    start([cp_w(16)])
    for q in range(len(XS)):
        start(cp_x0(q))
    start([cp_w(9)])
    start([cp_w(17)])
    start([cp_phi1])
    for g in range(2, 8):
        start([cp_w(8 + g)])
        start([cp_w(16 + g)])
    for t in range(1, NT_):
        start(cp_x(t))
    start([cp_w(g) for g in range(8)])
    start(cp_wo)

    row = lax.broadcasted_iota(jnp.int32, (128, 128), 0)
    col = lax.broadcasted_iota(jnp.int32, (128, 128), 1)
    bdmask = (row // 32) == (col // 32)

    def make_bd(g):
        w4 = wphis[4 * g:4 * g + 4].astype(F32).reshape(128, 32)
        bdT = jnp.where(bdmask, jnp.concatenate([w4] * 4, axis=1), 0.0).T
        for pj in range(2):
            for hh in range(2):
                r = 64 * pj + 32 * hh
                bscr[g % 2, pl.ds(64 * pj + hh, 32, stride=2), :] = bdT[r:r + 32, :]
        bds[g] = bscr[g % 2].astype(BF16)

    def fold(c, g, r0):
        put_wT(r0, (_dot_nt(bds[g], wst[c]) * LOG2E).astype(BF16))

    def trans_v(g):
        put_wT(vr(g), wst[16 + g].T)

    def feat_k(p, r0, first):
        for j in range(p.shape[0] // 64):
            ep, en, rp, rn = _softpm(p[64 * j:64 * j + 64, :])
            for e, r, o in ((ep, rp, 0), (en, rn, 64)):
                f = e * _rep(r, 8)
                a = r0 + 128 * j + o
                put_phi(a, f)
                zp = f[:, 0:128]
                for l in range(1, NL):
                    zp = zp + f[:, 128 * l:128 * l + 128]
                zacc[a:a + 64, :] = zp if first else zacc[a:a + 64, :] + zp

    def feat_q(p, r0):
        for j in range(p.shape[0] // 64):
            ep, en, rp, rn = _softpm(p[64 * j:64 * j + 64, :])
            a = r0 + 128 * j
            tp = _tree(jnp.add, _vregs(ep * _lcat([zacc[a:a + 64, :]] * NL)))
            tn = _tree(jnp.add, _vregs(en * _lcat([zacc[a + 64:a + 128, :]] * NL)))
            den = tp * rp + tn * rn
            for sh in (4, 2):
                den = den + pltpu.roll(den, sh, 0)
            rd = _rcp(den + 1e-6)
            put_phi(a, ep * _rep(rp * rd, 8))
            put_phi(a + 64, en * _rep(rn * rd, 8))

    def store_v(v, g):
        v = v.astype(BF16)
        for jj in range(2):
            lhs[2 * g + jj] = v[64 * jj:64 * jj + 64, :]

    def kv_dot(j):
        return _dot_nt(lhs[j], get_phi(j))

    wait([cp_phi0])
    for g in range(3):
        make_bd(g)
    wait([cp_w(8)])
    fold(8, 0, kr(0))
    wait([cp_w(16)])
    trans_v(0)
    p = None
    for q in range(len(XS)):
        wait(cp_x0(q))
        xq = _lcat([xs[j, 0:TS, :] for j in XS[q]])
        pq = _dot_nt(wrows(kr(0), 256)[:, 128 * XS[q][0]:128 * XS[q][-1] + 128], xq)
        p = pq if p is None else p + pq
    store_v(p[128:256], 0)
    p = p[0:128]
    for g in range(1, 8):
        if g == 1:
            wait([cp_w(9)])
        elif g == 2:
            wait([cp_w(17), cp_phi1, cp_w(10)])
        elif g == 3:
            wait([cp_w(18), cp_w(11), cp_w(19), cp_w(12)])
        elif g == 5:
            wait([cp_w(c) for c in (20, 21, 22, 23, 13, 14, 15)])
        fold(8 + g, g, kr(g))
        if g > 1:
            trans_v(g - 1)
            store_v(_dot_nt(wrows(vr(g - 1), 128), xtile(0)), g - 1)
        feat_k(p, 256 * (g - 1), True)
        if g == 2:
            for gg in range(3, 8):
                make_bd(gg)
        p = _dot_nt(wrows(kr(g), 128), xtile(0))
    xu[0:TS // 2, :] = _pk(xtile(0))
    trans_v(7)
    store_v(_dot_nt(wrows(vr(7), 128), xtile(0)), 7)
    feat_k(p, 256 * 7, True)
    for j in range(16):
        acc[j] = kv_dot(j)

    def ph1(t, _):
        wait(cp_x(t))
        xt = xtile(pl.multiple_of(t * TS, TS))
        xu[pl.ds(pl.multiple_of(t * (TS // 2), TS // 2), TS // 2), :] = _pk(xt)
        for g in range(8):
            pv = _dot_nt(wrows(kr(g), 256), xt)
            feat_k(pv[0:128], 256 * g, False)
            store_v(pv[128:256], g)
        for j in range(16):
            acc[j] = acc[j] + kv_dot(j)
        return 0

    lax.fori_loop(1, NT_, ph1, 0)

    wait([cp_w(g) for g in range(8)])
    wait(cp_wo)
    ones = jnp.ones((16, 128), BF16)
    for j in range(16):
        zr = _dot_nt(ones, zacc[128 * j:128 * j + 128, :].astype(BF16))
        zacc[128 * j:128 * j + 128, :] = _rep(zr, 8).T
    for g in range(8):
        fold(g, g, 128 * g)
    rr = lax.broadcasted_iota(jnp.int32, (64, 128), 0)
    cc = lax.broadcasted_iota(jnp.int32, (64, 128), 1)
    amask = (rr // 32) == (cc % 2)
    for j in range(16):
        amat[j] = jnp.where(amask, acc[j], 0.0).astype(BF16)

    def ph2(t, _):
        s0 = pl.multiple_of(t * TS, TS)
        xt = _upk(xu[pl.ds(pl.multiple_of(t * (TS // 2), TS // 2), TS // 2), :])
        for g in range(8):
            feat_q(_dot_nt(wrows(128 * g, 128), xt), 256 * g)
        for j in range(16):
            oT[64 * j:64 * j + 64, :] = _dot_nn(amat[j], get_phi(j)).astype(BF16)
        o = oT[...].T
        for c in range(8):
            ost[pl.ds(s0, TS), 128 * c:128 * c + 128] = _dot_nn(o, wos[c]).astype(BF16)
            cp_o(t, c).start()
        return 0

    lax.fori_loop(0, NT_, ph2, 0)
    pltpu.make_async_copy(ost, ost, sems.at[S_OUT]).wait()


@jax.jit
def pallas_standalone__linear_kernel_hedgehog__prompt_kernel(x, wqkv, w_phi, wo):
    anyspec = pl.BlockSpec(memory_space=pl.ANY)
    out = pl.pallas_call(
        _kernel,
        out_shape=jax.ShapeDtypeStruct((S, D), BF16),
        in_specs=[anyspec] * 4,
        out_specs=anyspec,
        scratch_shapes=[
            pltpu.VMEM((8, S, 128), BF16),
            pltpu.VMEM((24, D, 128), BF16),
            pltpu.VMEM((H, DH, DH), BF16),
            pltpu.VMEM((8, D, 128), BF16),
            pltpu.VMEM((3 * D // 2, D), U32),
            pltpu.VMEM((8, 128, 128), BF16),
            pltpu.VMEM((2, 128, 128), F32),
            pltpu.VMEM((16, 64, 128), F32),
            pltpu.VMEM((16, 64, 128), BF16),
            pltpu.VMEM((16, 64, TS), BF16),
            pltpu.VMEM((D, TS), U32),
            pltpu.VMEM((D, TS), BF16),
            pltpu.VMEM((S, D), BF16),
            pltpu.VMEM((2 * D, 128), F32),
            pltpu.VMEM((S // 2, D), U32),
            pltpu.SemaphoreType.DMA((N_SEM,)),
            pltpu.SemaphoreType.REGULAR,
        ],
        compiler_params=pltpu.CompilerParams(vmem_limit_bytes=100 * 1024 * 1024, disable_semaphore_checks=True),
    )(x.reshape(S, D), wqkv, w_phi, wo)
    return out.reshape(1, S, D)
```
